```python
import os as _os
_os.environ.setdefault("JAX_PLATFORMS", "cpu")
import jax
import jax.numpy as jnp

def _softmax(x, axis=-1):
    return jax.nn.softmax(x, axis=axis)
def _gelu(x):
    return jax.nn.gelu(x, approximate=True)
def _silu(x):
    return jax.nn.silu(x)
def _sigmoid(x):
    return jax.nn.sigmoid(x)
def _layernorm(x, axis=-1, eps=1e-5):
    m = jnp.mean(x, axis=axis, keepdims=True)
    v = jnp.var(x, axis=axis, keepdims=True)
    return (x - m) / jnp.sqrt(v + eps)
def _scatter_add(tgt, idx, src, axis=0):
    return tgt.at[idx].add(src)
def _segment_sum(src, seg, n):
    return jax.ops.segment_sum(src, seg, n)
class _Rng:
    def __init__(self, key):
        self._k = key
    def _next(self):
        self._k, sub = jax.random.split(self._k)
        return sub
    def normal(self, shape):
        return jax.random.normal(self._next(), shape, dtype=jnp.bfloat16)
    def randint(self, lo, hi, shape):
        return jax.random.randint(self._next(), shape, lo, hi, dtype=jnp.int32)
    def uniform(self, shape, lo=0.0, hi=1.0):
        return jax.random.uniform(self._next(), shape, jnp.bfloat16, lo, hi)
    def permutation(self, n):
        return jax.random.permutation(self._next(), n)


kernel_name = 'concat_heads__mha_block__ssm_conv_s4__prompt'

def setup_inputs():
    _rng = _Rng(jax.random.key(int.from_bytes(__import__("os").urandom(4), "little")))
    _w = (lambda a: (lambda t: t.astype(jnp.bfloat16) if jnp.issubdtype(t.dtype, jnp.floating) else t)(jnp.asarray(a)))
    def _A_setup():
        B, S, D, H = 1, 2048, 448, 16
        return {
            "x": _w((lambda *s: _rng.normal(s) * 0.2)(B, S, D)),
            "wqkv": _w((lambda *s: _rng.normal(s) * 0.2)(D, 3 * D)),
            "wo": _w((lambda *s: _rng.normal(s) * 0.05)(D, D)),
        }
    _A_in = _A_setup()

    def _B_setup():
        B, L, D, N = 1, 2048, 448, 256
        A_re = -jnp.exp((lambda *s: _rng.normal(s) * 0.2)(D, N))
        A_im = jnp.pi * (lambda *s: _rng.normal(s) * 0.2)(D, N)
        B_re = (lambda *s: _rng.normal(s) * 0.2)(D, N)
        B_im = (lambda *s: _rng.normal(s) * 0.2)(D, N)
        C_re = (lambda *s: _rng.normal(s) * 0.2)(D, N)
        C_im = (lambda *s: _rng.normal(s) * 0.2)(D, N)
        log_dt = (lambda *s: _rng.normal(s) * 0.2)(D) * 0.5 - 4.0
        Dskip = (lambda *s: _rng.normal(s) * 0.05)(D)
        return {
            "u": _w((lambda *s: _rng.normal(s) * 0.05)(B, L, D)),
            "A_re": _w(A_re),
            "A_im": _w(A_im),
            "B_re": _w(B_re),
            "B_im": _w(B_im),
            "C_re": _w(C_re),
            "C_im": _w(C_im),
            "log_dt": _w(log_dt),
            "Dskip": _w(Dskip),
        }
    _B_in = _B_setup()

    return {
        "A_x": _A_in["x"],
        "A_wqkv": _A_in["wqkv"],
        "A_wo": _A_in["wo"],
        "B_u": _B_in["u"],
        "B_A_re": _B_in["A_re"],
        "B_A_im": _B_in["A_im"],
        "B_B_re": _B_in["B_re"],
        "B_B_im": _B_in["B_im"],
        "B_C_re": _B_in["C_re"],
        "B_C_im": _B_in["C_im"],
        "B_log_dt": _B_in["log_dt"],
        "B_Dskip": _B_in["Dskip"],
    }

def reference(A_x, A_wqkv, A_wo, B_u, B_A_re, B_A_im, B_B_re, B_B_im, B_C_re, B_C_im, B_log_dt, B_Dskip):
    def _A_ref(x, wqkv, wo):
        B, S, D = x.shape
        H = 16
        Dh = D // H
        qkv = (lambda x, *d: x.transpose(*d))((x @ wqkv).reshape(B, S, 3, H, Dh), 2, 0, 3, 1, 4)
        q, k, v = qkv[0], qkv[1], qkv[2]
        scores = jnp.einsum("bhqd,bhkd->bhqk", q, k) * (Dh ** -0.5)
        p = _softmax(scores, axis=-1)
        o = jnp.einsum("bhqk,bhkd->bhqd", p, v)
        return (lambda x, *d: x.transpose(*d))(o, 0, 2, 1, 3).reshape(B, S, D) @ wo

    def _B_ref(u, A_re, A_im, B_re, B_im, C_re, C_im, log_dt, Dskip):
        Bsz, L, D = u.shape
        dt = jnp.exp(log_dt)[:, None]
        A = A_re + 1j * A_im
        Bc = B_re + 1j * B_im
        Cc = C_re + 1j * C_im
        logdA = dt * A
        dB = dt * Bc
        l = (lambda x, dt: x.astype(dt))(jnp.arange(L), A_re.dtype)
        P = jnp.exp(logdA[:, :, None] * l[None, None, :])
        K = jnp.einsum("dn,dnl,dn->dl", Cc, P, dB).real
        L2 = 2 * L
        Kp = jnp.pad(K, ((0, 0), (0, L)))
        up = (lambda x, *d: x.transpose(*d))(u, 0, 2, 1)
        up = jnp.pad(up, ((0, 0), (0, 0), (0, L)))
        Kf = (lambda x, axes=(-2,-1): jnp.fft.rfft2(x.astype(jnp.float32), axes=axes))(Kp[:, None, :], axes=(-2, -1))
        Uf = (lambda x, axes=(-2,-1): jnp.fft.rfft2(x.astype(jnp.float32), axes=axes))(up[:, :, None, :], axes=(-2, -1))
        Yf = Uf * Kf[None, :, :, :]
        y = (lambda x, s, axes=(-2,-1): jnp.fft.irfft2(x, s=s, axes=axes).astype(jnp.bfloat16))(Yf, (1, L2), axes=(-2, -1))[:, :, 0, :L]
        y = (lambda x, *d: x.transpose(*d))(y, 0, 2, 1) + u * Dskip[None, None, :]
        return y

    a = _A_ref(A_x, A_wqkv, A_wo)
    b = _B_ref(B_u, B_A_re, B_A_im, B_B_re, B_B_im, B_C_re, B_C_im, B_log_dt, B_Dskip)
    return jnp.concatenate([a, b], axis=-1)
```

```python
import numpy as np
import jax
import jax.numpy as jnp
from jax import lax
import jax.experimental.pallas as pl
import jax.experimental.pallas.tpu as pltpu

S = 2048
D = 448
H = 16
DH = 28
N = 256
DP = 512
BQ = 512
CK = 128
NB = 16
f32 = jnp.float32
bf16 = jnp.bfloat16

HI = (0, 1, 2, 3, 256, 258, 512, 768, 1024, 1280, 1536, 1792, 2048)
LO_STEP = 4
NLO = 64
ES = 9
HS = 13
RS = 17


def _bf16_round(x):
    u = np.asarray(x, np.float32).view(np.uint32).astype(np.uint64)
    u = (u + 0x7FFF + ((u >> 16) & 1)) & 0xFFFF0000
    return u.astype(np.uint32).view(np.float32)


def _conv_constants():
    lr = _bf16_round(np.arange(S)).astype(np.int64)
    f = np.arange(128)
    ktile = NLO * 2
    fk = np.zeros((NB, 256, 16 * NLO))
    for p in range(NB):
        for tau in range(-127, 128):
            l = 128 * p + tau
            if 0 <= l < S:
                lp = int(lr[l])
                col = None
                for rho, hi in enumerate(HI):
                    if lp >= hi and (lp - hi) % LO_STEP == 0 and (lp - hi) // LO_STEP < NLO:
                        col = rho * NLO + (lp - hi) // LO_STEP
                        break
                assert col is not None
                ang = np.pi * (2 * f + 1) * tau / 256
                fk[p, :128, col] += np.cos(ang)
                fk[p, 128:, col] -= np.sin(ang)
    tiles, index = [], []
    for p in range(NB):
        mine = []
        for kt in range(fk.shape[2] // ktile):
            blk = fk[p, :, kt * ktile:(kt + 1) * ktile]
            if np.any(blk != 0):
                mine.append((len(tiles), kt))
                tiles.append(blk)
        index.append(tuple(mine))
    ang = np.pi * np.outer(2 * f + 1, np.arange(128)) / 256
    fu = np.concatenate([np.cos(ang), -np.sin(ang)], axis=0)
    gi = np.concatenate([np.cos(ang.T), -np.sin(ang.T)], axis=1) / 128
    gi = gi.reshape(128, 2, 8, 16).transpose(0, 2, 1, 3).reshape(128, 256)
    return np.stack(tiles), tuple(index), fu, gi


_FK, _FK_INDEX, _FU, _GI = _conv_constants()
_NFK = _FK.shape[0]


def _cmul(a, b):
    return a[0] * b[0] - a[1] * b[1], a[0] * b[1] + a[1] * b[0]


def _csq(a):
    t = a[0] * a[1]
    return a[0] * a[0] - a[1] * a[1], t + t


def _respace(w, base):
    z = jnp.zeros((32 - DH, w.shape[1]), w.dtype)
    parts = []
    for h in range(H):
        parts += [w[base + DH * h: base + DH * (h + 1)], z]
    return jnp.concatenate(parts, axis=0)


(SEM_W, SEM_X, SEM_P, SEM_DT, SEM_DS, SEM_U, SEM_WO, SEM_FU, SEM_GI, SEM_FK, SEM_O) = (
    0, 1, 5, 11, 12, 13, 14, 15, 16, 17, 18)
N_SEM = SEM_O + NB


def _kernel(xt_hbm, wqkv_hbm, wo_hbm, ut_hbm, are_hbm, aim_hbm, bre_hbm, bim_hbm,
            cre_hbm, cim_hbm, ldt_hbm, dskip_hbm, fu_hbm, gi_hbm, fk_hbm,
            out_hbm,
            wraw, wo_raw, xs, pbuf, ldt_v, dskip_v, fu_ref, gi_ref, fk_ref,
            wqv, wk, wo2, kp, qt, vt, s_ref, ot,
            dtb, ebuf, hbuf, sbuf, rbuf, tm, us, kx, yb, ob, sems):
    def copy(src, dst, k):
        return pltpu.make_async_copy(src, dst, sems.at[k])

    c_w = copy(wqkv_hbm, wraw, SEM_W)
    c_x = [copy(xt_hbm.at[:, b * BQ:(b + 1) * BQ], xs.at[0:D, b * BQ:(b + 1) * BQ], SEM_X + b)
           for b in range(S // BQ)]
    c_p = [copy(r, pbuf.at[k], SEM_P + k)
           for k, r in enumerate((are_hbm, aim_hbm, bre_hbm, bim_hbm, cre_hbm, cim_hbm))]
    c_dt = copy(ldt_hbm, ldt_v, SEM_DT)
    c_ds = copy(dskip_hbm, dskip_v, SEM_DS)
    c_u = copy(ut_hbm, us.at[DP - D:DP, :], SEM_U)
    c_wo = copy(wo_hbm, wo_raw, SEM_WO)
    c_fu = copy(fu_hbm, fu_ref, SEM_FU)
    c_gi = copy(gi_hbm, gi_ref, SEM_GI)
    c_fk = copy(fk_hbm, fk_ref, SEM_FK)
    for c in [c_w, c_x[0], c_dt, c_x[1]] + c_p + c_x[2:] + [c_u, c_wo, c_ds, c_fu, c_gi, c_fk]:
        c.start()
    xs[D:DP, :] = jnp.zeros((DP - D, S), bf16)
    us[0:DP - D, :] = jnp.zeros((DP - D, S), bf16)
    for k in range(4):
        hbuf[k, pl.ds(HS * D, 8), :] = jnp.zeros((8, 128), f32)

    c_w.wait()
    wt = wraw[...].T.astype(f32)
    wt = jnp.concatenate([wt, jnp.zeros((3 * D, DP - D), f32)], axis=1)
    wqv[0:512, :] = _respace(wt, 0).astype(bf16)
    wqv[512:1024, :] = _respace(wt, 2 * D).astype(bf16)
    wk[...] = _respace(wt, D).T.astype(bf16)

    c_dt.wait()
    dt_row = jnp.exp(ldt_v[...].astype(f32).reshape(1, D)).astype(bf16).astype(f32)
    dtb[0:DP, :] = jnp.broadcast_to(
        jnp.concatenate([dt_row, jnp.zeros((1, DP - D), f32)], axis=1), (128, DP)).T

    def powers(groups):
        def pin(v, tile):
            return v + tile * 0.0

        for g in groups:
            d0 = pl.multiple_of(g * 16, 16)
            for k in range(2):
                ls = slice(128 * k, 128 * (k + 1))
                ar, ai, br, bi, cr, ci = [
                    pbuf[q, pl.ds(d0, 16), ls].astype(f32) for q in range(6)]
                for hf in range(2):
                    rs = slice(8 * hf, 8 * (hf + 1))
                    dd = d0 + 8 * hf

                    def st_e(s, z):
                        ebuf[k, pl.ds(ES * dd + s, 8, stride=ES), :] = z[0]
                        ebuf[2 + k, pl.ds(ES * dd + s, 8, stride=ES), :] = z[1]

                    def st_h(rho, w):
                        hbuf[k, pl.ds(HS * dd + rho, 8, stride=HS), :] = w[0]
                        hbuf[2 + k, pl.ds(HS * dd + rho, 8, stride=HS), :] = -w[1]

                    dt = pin(dtb[pl.ds(dd, 8), :], (yield))
                    a = dt * ar[rs]
                    b = dt * ai[rs]
                    w0 = _cmul((cr[rs], ci[rs]), (dt * br[rs], dt * bi[rs]))
                    ea = jnp.exp(a)
                    b = pin(b, (yield))
                    z1 = (ea * jnp.cos(b), ea * jnp.sin(b))
                    z1 = (pin(z1[0], (yield)), z1[1])
                    z2 = _csq(z1)
                    st_h(0, w0)
                    w = w0
                    for rho in (1, 2, 3):
                        w = _cmul(w, z1)
                        st_h(rho, w)
                    z4 = _csq(z2)
                    st_e(0, (jnp.ones((8, 128), f32), jnp.zeros((8, 128), f32)))
                    st_e(1, z4)
                    e = (pin(z4[0], (yield)), z4[1])
                    for sidx in range(2, 5):
                        e = _cmul(e, z4)
                        st_e(sidx, e)
                    e = (pin(e[0], (yield)), e[1])
                    for sidx in range(5, 8):
                        e = _cmul(e, z4)
                        st_e(sidx, e)
                    z32 = _cmul(e, z4)
                    sbuf[k, pl.ds(dd, 8), :] = z32[0]
                    sbuf[2 + k, pl.ds(dd, 8), :] = z32[1]
                    z32 = (pin(z32[0], (yield)), z32[1])
                    z256 = _csq(_csq(_csq(z32)))
                    w = _cmul(w0, z256)
                    st_h(4, w)
                    st_h(5, _cmul(w, z2))
                    w = (pin(w[0], (yield)), w[1])
                    for rho in range(6, 10):
                        w = _cmul(w, z256)
                        st_h(rho, w)
                    w = (pin(w[0], (yield)), w[1])
                    for rho in range(10, 13):
                        w = _cmul(w, z256)
                        st_h(rho, w)

    def tap_pair(i):
        d = 2 * i

        def ld2(buf, k, pitch, n):
            return jnp.concatenate([buf[k, pl.ds(pitch * d, n), :],
                                    buf[k, pl.ds(pitch * (d + 1), n), :]], axis=0)

        def bc2(k):
            return jnp.concatenate(
                [jnp.broadcast_to(sbuf[k, pl.ds(d + t, 1), :], (8, 128)) for t in range(2)], axis=0)

        zs = [[None] * 4 for _ in range(8)]
        for k in range(2):
            z = (ld2(ebuf, k, ES, 8), ld2(ebuf, 2 + k, ES, 8))
            step = (bc2(k), bc2(2 + k))
            for g in range(8):
                zs[g][k], zs[g][2 + k] = z
                if g < 7:
                    z = _cmul(z, step)
        lo = jnp.concatenate([jnp.concatenate(zs[g], axis=1) for g in range(8)], axis=0).astype(bf16)
        hi = jnp.concatenate([ld2(hbuf, k, HS, 16) for k in range(4)], axis=1).astype(bf16)
        res = lax.dot_general(hi, lo, (((1,), (1,)), ((), ())), preferred_element_type=f32)
        rbuf[pl.ds(RS * d, 16), :] = res[0:16]
        rbuf[pl.ds(RS * (d + 1), 16), :] = res[16:32]

    qscale = float(DH ** -0.5 * np.log2(np.e))
    row = lax.broadcasted_iota(jnp.int32, (128, BQ), 0)
    gpi = (D // 16) // (S // BQ)

    n_stage = 8 * 4 * gpi
    n_skip = 4 * 32
    n_mark = 12 * 32 - n_skip

    def proj(tb, carry):
        ts = pl.ds(pl.multiple_of(tb * BQ, BQ), BQ)
        pltpu.make_async_copy(xt_hbm.at[:, ts], xs.at[0:D, ts], sems.at[SEM_X + tb]).wait()
        job = powers([tb * gpi + g for g in range(gpi)])
        cnt = {"mark": 0, "stage": 0}

        def pace(val):
            for g in range(val.shape[0] // 16):
                cnt["mark"] += 1
                m = cnt["mark"] - n_skip
                if m == 1:
                    @pl.when(tb == 0)
                    def _():
                        for c in c_p:
                            c.wait()
                    next(job)
                while m > 0 and cnt["stage"] < (m * n_stage + n_mark - 1) // n_mark:
                    cnt["stage"] += 1
                    try:
                        job.send(val[16 * g:16 * g + 8, 0:128])
                    except StopIteration:
                        pass

        for g in range(8):
            r = None
            for kt in range(4):
                ks = slice(128 * kt, 128 * (kt + 1))
                part = jnp.dot(wqv[128 * g:128 * (g + 1), ks], xs[ks, ts], preferred_element_type=f32)
                r = part if r is None else r + part
                pace(part)
            if g < 4:
                qt[g, :, ts] = (r * qscale).astype(bf16)
            else:
                v = jnp.where((row & 31) == DH, 1.0, r).astype(bf16)
                for hh in range(4):
                    vt[4 * (g - 4) + hh, :, ts] = v[32 * hh:32 * (hh + 1)]
            if g % 2 == 1:
                tt = g // 2
                tsl = pl.ds(pl.multiple_of(tb * BQ + 128 * tt, 128), 128)
                k = None
                for kt in range(4):
                    ks = slice(128 * kt, 128 * (kt + 1))
                    part = lax.dot_general(xs[ks, tsl], wk[ks, :], (((0,), (0,)), ((), ())),
                                           preferred_element_type=f32)
                    k = part if k is None else k + part
                    pace(part)
                kb = k.astype(bf16)
                for c in range(4):
                    kp[c, tsl, :] = kb[:, 128 * c:128 * (c + 1)]
        assert cnt["stage"] == n_stage
        return carry

    lax.fori_loop(0, S // BQ, proj, 0)

    nq = S // BQ
    nc = S // CK

    def masked_q(c, q0, j):
        parts = []
        if j > 0:
            parts.append(jnp.zeros((32 * j, BQ), bf16))
        parts.append(qt[c, 32 * j:32 * (j + 1), pl.ds(q0, BQ)])
        if j < 3:
            parts.append(jnp.zeros((32 * (3 - j), BQ), bf16))
        return jnp.concatenate(parts, axis=0)

    def unit(i):
        return i // nq, pl.multiple_of((i % nq) * BQ, BQ)

    qm = masked_q(0, 0, 0)
    mp = None
    for kc in range(nc):
        sl = slice(kc * CK, (kc + 1) * CK)
        s = jnp.dot(kp[0, sl, :], qm, preferred_element_type=f32)
        s_ref[0, sl, :] = s
        cm = jnp.max(s.reshape(CK // 8, 8, BQ), axis=0)
        mp = cm if mp is None else jnp.maximum(mp, cm)
    m0 = jnp.max(mp, axis=0, keepdims=True)

    n_it = 4 * nq
    s_ref[1, S - CK:S, :] = jnp.zeros((CK, BQ), f32)

    def pv(slot, h, kc, m, acc):
        sl = slice(kc * CK, (kc + 1) * CK)
        p = jnp.exp2(s_ref[slot, sl, :] - m).astype(bf16)
        o = jnp.dot(vt[h, :, sl], p, preferred_element_type=f32)
        return o if acc is None else acc + o

    def normalise(h, q0, acc):
        inv = 1.0 / acc[DH:DH + 1]
        ot[pl.ds(pl.multiple_of(h * 32, 32), 32), pl.ds(q0, BQ)] = (acc * inv).astype(bf16)

    def att(side_job, i, carry, last=False):
        m_cur, m_prev, acc = carry
        state = {}
        for j in range(4):
            c, q0 = unit(i)
            h = c * 4 + j
            if j > 0:
                hp, q0p = h - 1, q0
            else:
                cp, q0p = unit(jnp.maximum(i - 1, 0))
                hp = cp * 4 + 3
            do_qk = not (last and j == 3)
            if j < 3:
                cn, q0n, jn = c, q0, j + 1
            else:
                cn, q0n = unit(jnp.minimum(i + 1, n_it - 1))
                jn = 0
            slot, nslot = j % 2, (j + 1) % 2
            if do_qk:
                qm = masked_q(cn, q0n, jn)
            mp = None
            for kc in range(nc):
                if do_qk:
                    sl = slice(kc * CK, (kc + 1) * CK)
                    s = jnp.dot(kp[cn, sl, :], qm, preferred_element_type=f32)
                    s_ref[nslot, sl, :] = s
                    cm = jnp.max(s.reshape(CK // 8, 8, BQ), axis=0)
                    mp = cm if mp is None else jnp.maximum(mp, cm)
                    side_job(i, j * nc + kc, s, state)
                if kc == 0:
                    normalise(hp, q0p, pv(nslot, hp, nc - 1, m_prev, acc))
                    acc = None
                else:
                    acc = pv(slot, h, kc - 1, m_cur, acc)
            m_prev = m_cur
            if do_qk:
                m_cur = jnp.max(mp, axis=0, keepdims=True)
        if last:
            normalise(h, q0, pv(1, h, nc - 1, m_prev, acc))
        return m_cur, m_prev, acc

    n_a = n_it // 2
    ppi = (D // 2) // n_a
    pair_at = {(k * 64) // ppi: k for k in range(ppi)}

    def tap_job(i, ci, s, state):
        if ci in pair_at:
            tap_pair(i * ppi + pair_at[ci])

    carry = (m0, jnp.zeros((1, BQ), f32), jnp.zeros((32, BQ), f32))
    carry = lax.fori_loop(0, n_a, lambda i, m: att(tap_job, i, m), carry)

    c_ds.wait()
    c_wo.wait()
    wo_r = _respace(wo_raw[...].astype(f32), 0)
    wo2[...] = jnp.concatenate([wo_r, jnp.zeros((512, DP - D), f32)], axis=1).astype(bf16)
    dsk = jnp.concatenate([jnp.zeros((1, DP - D), f32),
                           dskip_v[...].astype(f32).reshape(1, D)], axis=1)
    odd = (lax.broadcasted_iota(jnp.int32, (8, DP), 1) & 1) == 1
    first = lax.broadcasted_iota(jnp.int32, (8, DP), 0) == 0
    for rho in range(len(HI)):
        m = jnp.concatenate([jnp.zeros((DP - D, 128), f32),
                             rbuf[pl.ds(rho, D, stride=RS), :]], axis=0)
        mt = m.T
        rows = [jnp.where(odd, mt[16 * g + 8:16 * g + 16], mt[16 * g:16 * g + 8]) for g in range(8)]
        if rho == 0:
            rows[0] = rows[0] + jnp.where(first, dsk, 0.0)
        tm[NLO * rho:NLO * (rho + 1), :] = jnp.concatenate(rows, axis=0).astype(bf16)
    tm[NLO * len(HI):NLO * 14, :] = jnp.zeros((NLO, DP), bf16)

    for c in (c_u, c_fu, c_gi, c_fk):
        c.wait()

    def put_spectrum(slab, r):
        for g in range(16):
            for t in range(4):
                r0 = 32 * t + 16 * (g // 8) + (8 if slab >= NB else 0)
                kx[g % 8, slab, r0:r0 + 16, :] = r[16 * g:16 * (g + 1), 128 * t:128 * (t + 1)]

    for j in range(NB):
        put_spectrum(NB + j, lax.dot_general(
            fu_ref[...], us[:, 128 * j:128 * (j + 1)], (((1,), (1,)), ((), ())),
            preferred_element_type=f32))
        r = None
        for idx, kt in _FK_INDEX[j]:
            part = jnp.dot(fk_ref[idx], tm[128 * kt:128 * (kt + 1), :], preferred_element_type=f32)
            r = part if r is None else r + part
        put_spectrum(j, r)

    units = [(t, io, hf, p) for t in range(4) for io in range(NB) for hf in range(2)
             for p in range(io + 1)]

    def mac_job(i, ci, s, state, n_chunks=64):
        fg = i - n_a
        mine = units[(ci * len(units)) // n_chunks:((ci + 1) * len(units)) // n_chunks]
        for m, (t, io, hf, p) in enumerate(mine):
            g = (m * 8) // len(mine)
            r0 = 32 * t + 8 * hf
            kr, ki = kx[fg, p, r0:r0 + 8, :], kx[fg, p, r0 + 16:r0 + 24, :]
            ur = kx[fg, NB + io - p, r0 + 8:r0 + 16, :]
            ui = kx[fg, NB + io - p, r0 + 24:r0 + 32, :]
            if m == 0 or ((m - 1) * 8) // len(mine) != g:
                kr = kr + s[16 * g:16 * g + 8, 0:128] * 0.0
            a = kr * ur - ki * ui
            b = kr * ui + ki * ur
            if p == 0:
                state["re"], state["im"] = a, b
            else:
                state["re"], state["im"] = state["re"] + a, state["im"] + b
            if p == io:
                if hf == 0:
                    state["re0"], state["im0"] = state["re"], state["im"]
                else:
                    ls = slice(128 * t, 128 * (t + 1))
                    y0 = pl.multiple_of(fg * 32, 32)
                    yb[io, pl.ds(y0, 16), ls] = jnp.concatenate(
                        [state["re0"], state["re"]], axis=0).astype(bf16)
                    yb[io, pl.ds(y0 + 16, 16), ls] = jnp.concatenate(
                        [state["im0"], state["im"]], axis=0).astype(bf16)

    carry = lax.fori_loop(n_a, n_it - 1, lambda i, m: att(mac_job, i, m), carry)
    att(lambda i, ci, s, st: mac_job(i, ci, s, st, 48), n_it - 1, carry, last=True)

    lane = lax.broadcasted_iota(jnp.int32, (128, 128), 1)
    for i in range(NB):
        rows = slice(128 * i, 128 * (i + 1))
        y = jnp.dot(gi_ref[...], yb[i], preferred_element_type=f32)
        a = lax.dot_general(ot[:, rows], wo2[...], (((0,), (0,)), ((), ())),
                            preferred_element_type=f32)
        ob[rows, 0:384] = a[:, 0:384].astype(bf16)
        ob[rows, 384:512] = jnp.where(lane < 64, a[:, 384:512], y[:, 0:128]).astype(bf16)
        ob[rows, 512:896] = y[:, 128:512].astype(bf16)
        copy(ob.at[rows, :], out_hbm.at[rows, :], SEM_O + i).start()
    for i in range(NB):
        rows = slice(128 * i, 128 * (i + 1))
        copy(ob.at[rows, :], out_hbm.at[rows, :], SEM_O + i).wait()


@jax.jit
def pallas_concat_heads__mha_block__ssm_conv_s4__prompt_kernel(
    A_x: jax.Array,
    A_wqkv: jax.Array,
    A_wo: jax.Array,
    B_u: jax.Array,
    B_A_re: jax.Array,
    B_A_im: jax.Array,
    B_B_re: jax.Array,
    B_B_im: jax.Array,
    B_C_re: jax.Array,
    B_C_im: jax.Array,
    B_log_dt: jax.Array,
    B_Dskip: jax.Array,
):
    vm = pltpu.VMEM
    scratch = [
        vm((D, 3 * D), bf16), vm((D, D), bf16), vm((DP, S), bf16), vm((6, D, N), bf16),
        vm((D,), bf16), vm((D,), bf16), vm((256, 128), bf16), vm((128, 256), bf16),
        vm((_NFK, 256, 128), bf16),
        vm((1024, DP), bf16), vm((DP, 512), bf16), vm((512, DP), bf16),
        vm((4, S, 128), bf16), vm((4, 128, S), bf16), vm((H, 32, S), bf16),
        vm((2, S, BQ), f32), vm((512, S), bf16),
        vm((DP, 128), f32), vm((4, ES * D + 8, 128), f32), vm((4, HS * D + 8, 128), f32),
        vm((4, D, 128), f32), vm((RS * D + 8, 128), f32), vm((14 * NLO, DP), bf16),
        vm((DP, S), bf16), vm((8, 2 * NB, 160, 128), f32),
        vm((NB, 256, DP), bf16), vm((S, 2 * D), bf16),
        pltpu.SemaphoreType.DMA((N_SEM,)),
    ]
    hbm = pl.BlockSpec(memory_space=pl.ANY)
    out = pl.pallas_call(
        _kernel,
        out_shape=jax.ShapeDtypeStruct((S, 2 * D), bf16),
        in_specs=[hbm] * 15,
        out_specs=hbm,
        scratch_shapes=scratch,
        compiler_params=pltpu.CompilerParams(vmem_limit_bytes=110 * 1024 * 1024),
    )(jnp.transpose(A_x, (0, 2, 1)).reshape(D, S), A_wqkv, A_wo,
      jnp.transpose(B_u, (0, 2, 1)).reshape(D, S),
      B_A_re, B_A_im, B_B_re, B_B_im, B_C_re, B_C_im, B_log_dt, B_Dskip,
      jnp.asarray(_FU, bf16), jnp.asarray(_GI, bf16), jnp.asarray(_FK, bf16))
    return out.reshape(1, S, 2 * D)
```

```python
import numpy as np
import jax
import jax.numpy as jnp
from jax import lax
import jax.experimental.pallas as pl
import jax.experimental.pallas.tpu as pltpu

S = 2048
D = 448
H = 16
DH = 28
N = 256
DP = 512
BQ = 512
CK = 128
NB = 16
f32 = jnp.float32
bf16 = jnp.bfloat16

HI = (0, 1, 2, 3, 256, 258, 512, 768, 1024, 1280, 1536, 1792, 2048)
LO_STEP = 4
NLO = 64
ES = 9
HS = 13
RS = 17

PINS = (0, 1, 2, 3, 4, 5, 6, 7)
NSKIP = 212
G_FIRST = 4
MAC_PINS = 4
FILL_AT = (1, 6, 11)
MAC_SKIP = 2
FLAGS = {"XLA_TPU_EVENLY_DISTRIBUTE_CRITICAL_NODES": True}


def _bf16_round(x):
    u = np.asarray(x, np.float32).view(np.uint32).astype(np.uint64)
    u = (u + 0x7FFF + ((u >> 16) & 1)) & 0xFFFF0000
    return u.astype(np.uint32).view(np.float32)


def _slot(rho, unit):
    if rho < 4:
        return 8 * (unit // 2) + 2 * rho + unit % 2
    return 4 * rho + unit


def _conv_constants():
    lr = _bf16_round(np.arange(S)).astype(np.int64)
    f = np.arange(128)
    ktile = NLO * 2
    fk = np.zeros((NB, 256, 16 * NLO))
    for p in range(NB):
        for tau in range(-127, 128):
            l = 128 * p + tau
            if 0 <= l < S:
                lp = int(lr[l])
                col = None
                for rho, hi in enumerate(HI):
                    if lp >= hi and (lp - hi) % LO_STEP == 0 and (lp - hi) // LO_STEP < NLO:
                        q = (lp - hi) // LO_STEP
                        col = 16 * _slot(rho, q // 16) + q % 16
                        break
                assert col is not None
                ang = np.pi * (2 * f + 1) * tau / 256
                fk[p, :128, col] += np.cos(ang)
                fk[p, 128:, col] -= np.sin(ang)
    tiles, index = [], []
    for p in range(NB):
        mine = []
        for kt in range(fk.shape[2] // ktile):
            blk = fk[p, :, kt * ktile:(kt + 1) * ktile]
            if np.any(blk != 0):
                mine.append((len(tiles), kt))
                tiles.append(blk)
        index.append(tuple(mine))
    ang = np.pi * np.outer(2 * f + 1, np.arange(128)) / 256
    fu = np.concatenate([np.cos(ang), -np.sin(ang)], axis=0)
    gi = np.concatenate([np.cos(ang.T), -np.sin(ang.T)], axis=1) / 128
    gi = gi.reshape(128, 2, 8, 16).transpose(0, 2, 1, 3).reshape(128, 256)
    return np.stack(tiles), tuple(index), fu, gi


_FK, _FK_INDEX, _FU, _GI = _conv_constants()
_NFK = _FK.shape[0]


def _pack_host(a):
    u = _bf16_round(a).view(np.uint32) >> 16
    return (u[..., 0::2, :] | (u[..., 1::2, :] << 16)).astype(np.uint32).view(np.int32)


def _pack(x):
    return pltpu.bitcast(x.astype(bf16), jnp.int32)


def _unpack(w):
    return pltpu.bitcast(w, bf16)


def _cmul(a, b):
    return a[0] * b[0] - a[1] * b[1], a[0] * b[1] + a[1] * b[0]


def _cmul_conj(a, b):
    return a[0] * b[0] + a[1] * b[1], a[1] * b[0] - a[0] * b[1]


def _csq(a):
    t = a[0] * a[1]
    return a[0] * a[0] - a[1] * a[1], t + t


def _respace(w, base):
    z = jnp.zeros((32 - DH, w.shape[1]), w.dtype)
    parts = []
    for h in range(H):
        parts += [w[base + DH * h: base + DH * (h + 1)], z]
    return jnp.concatenate(parts, axis=0)


def _spread(r, pad):
    parts = []
    for h in range(4):
        parts += [r[DH * h:DH * (h + 1)], pad]
    return jnp.concatenate(parts, axis=0)


(SEM_W, SEM_X, SEM_P, SEM_DT, SEM_DS, SEM_U, SEM_WO, SEM_FU, SEM_GI, SEM_FK, SEM_O) = (
    0, 3, 7, 13, 14, 15, 16, 17, 18, 19, 20)
N_SEM = SEM_O + NB


def _kernel(xt_hbm, wqkv_hbm, wo_hbm, ut_hbm, are_hbm, aim_hbm, bre_hbm, bim_hbm,
            cre_hbm, cim_hbm, ldt_hbm, dskip_hbm, fu_hbm, gi_hbm, fk_hbm,
            out_hbm,
            wraw, wo_raw, xs, xi, pbuf, ldt_v, dskip_v, fu_ref, gi_ref, fk_ref,
            wqv, wk, wo2, kp, qt, vt, s_ref, ot,
            dtb, ebuf, hbuf, sbuf, rbuf, tm, us, kx, yb, ob, sems):
    def copy(src, dst, k):
        return pltpu.make_async_copy(src, dst, sems.at[k])

    w_cuts = ((0, 512), (896, 1344), (512, 896))
    c_w = [copy(wqkv_hbm.at[:, a:b], wraw.at[:, a:b], SEM_W + k) for k, (a, b) in enumerate(w_cuts)]
    c_x = [copy(xt_hbm.at[:, b * BQ:(b + 1) * BQ], xs.at[0:D, b * BQ:(b + 1) * BQ], SEM_X + b)
           for b in range(S // BQ)]
    c_p = [copy(r, pbuf.at[k], SEM_P + k)
           for k, r in enumerate((are_hbm, aim_hbm, bre_hbm, bim_hbm, cre_hbm, cim_hbm))]
    c_dt = copy(ldt_hbm, ldt_v, SEM_DT)
    c_ds = copy(dskip_hbm, dskip_v, SEM_DS)
    c_u = copy(ut_hbm, us.at[DP - D:DP, :], SEM_U)
    c_wo = copy(wo_hbm, wo_raw, SEM_WO)
    c_fu = copy(fu_hbm, fu_ref, SEM_FU)
    c_gi = copy(gi_hbm, gi_ref, SEM_GI)
    c_fk = copy(fk_hbm, fk_ref, SEM_FK)
    for c in (c_w[0], c_x[0], c_w[1], c_w[2]):
        c.start()
    c_dt.start()
    xs[D:DP, :] = jnp.zeros((DP - D, S), bf16)
    us[0:DP - D, :] = jnp.zeros((DP - D, S), bf16)
    for k in range(4):
        hbuf[k, pl.ds(HS * D, 8), :] = jnp.zeros((8, 128), f32)

    def w_rows(a, b):
        t = wraw[:, a:b].T.astype(f32)
        return jnp.concatenate([t, jnp.zeros((b - a, DP - D), f32)], axis=1)

    c_w[0].wait()
    t0 = w_rows(0, 512)
    wqv[0:D // 2, :] = _pack(t0[0:D])
    k_head = t0[D:512]

    def prep_v():
        c_w[1].wait()
        for c in c_p + [c_x[1]]:
            c.start()
        wqv[D // 2:D, :] = _pack(w_rows(896, 1344))

    def prep_k():
        c_w[2].wait()
        for c in c_x[2:] + [c_u, c_wo, c_ds, c_fu, c_gi, c_fk]:
            c.start()
        wkt = jnp.concatenate([k_head, w_rows(512, 896)], axis=0)
        wk[...] = _pack(_respace(wkt, 0).T)

    def prep_dt():
        c_dt.wait()
        dt_row = jnp.exp(ldt_v[...].astype(f32).reshape(1, D)).astype(bf16).astype(f32)
        dtb[0:DP, :] = jnp.broadcast_to(
            jnp.concatenate([dt_row, jnp.zeros((1, DP - D), f32)], axis=1), (128, DP)).T

    def powers(groups):
        def pin(v, tile):
            return v + tile * 0.0

        for g in groups:
            d0 = g * 16 if isinstance(g, int) else pl.multiple_of(g * 16, 16)
            for k in range(2):
                ls = slice(128 * k, 128 * (k + 1))
                ar, ai, br, bi, cr, ci = [
                    pbuf[q, pl.ds(d0, 16), ls].astype(f32) for q in range(6)]
                for hf in range(2):
                    rs = slice(8 * hf, 8 * (hf + 1))
                    dd = d0 + 8 * hf

                    def st_e(s, z):
                        ebuf[k, pl.ds(ES * dd + s, 8, stride=ES), :] = z[0]
                        ebuf[2 + k, pl.ds(ES * dd + s, 8, stride=ES), :] = z[1]

                    def st_h(rho, w):
                        hbuf[k, pl.ds(HS * dd + rho, 8, stride=HS), :] = w[0]
                        hbuf[2 + k, pl.ds(HS * dd + rho, 8, stride=HS), :] = w[1]

                    dt = dtb[pl.ds(dd, 8), :]
                    if 0 in PINS:
                        dt = pin(dt, (yield))
                    a = dt * ar[rs]
                    b = dt * ai[rs]
                    w0 = _cmul((cr[rs], ci[rs]), (dt * br[rs], dt * bi[rs]))
                    ea = jnp.exp(a)
                    if 1 in PINS:
                        b = pin(b, (yield))
                    z1 = (ea * jnp.cos(b), ea * jnp.sin(-b))
                    if 2 in PINS:
                        z1 = (pin(z1[0], (yield)), z1[1])
                    z2 = _csq(z1)
                    st_h(0, w0)
                    w = w0
                    for rho in (1, 2, 3):
                        w = _cmul_conj(w, z1)
                        st_h(rho, w)
                    z4 = _csq(z2)
                    st_e(0, (jnp.ones((8, 128), f32), jnp.zeros((8, 128), f32)))
                    st_e(1, z4)
                    e = z4
                    if 3 in PINS:
                        e = (pin(e[0], (yield)), e[1])
                    for sidx in range(2, 5):
                        e = _cmul(e, z4)
                        st_e(sidx, e)
                    if 4 in PINS:
                        e = (pin(e[0], (yield)), e[1])
                    for sidx in range(5, 8):
                        e = _cmul(e, z4)
                        st_e(sidx, e)
                    z32 = _cmul(e, z4)
                    sbuf[k, pl.ds(dd, 8), :] = z32[0]
                    sbuf[2 + k, pl.ds(dd, 8), :] = z32[1]
                    if 5 in PINS:
                        z32 = (pin(z32[0], (yield)), z32[1])
                    z256 = _csq(_csq(_csq(z32)))
                    w = _cmul_conj(w0, z256)
                    st_h(4, w)
                    st_h(5, _cmul_conj(w, z2))
                    if 6 in PINS:
                        w = (pin(w[0], (yield)), w[1])
                    for rho in range(6, 10):
                        w = _cmul_conj(w, z256)
                        st_h(rho, w)
                    if 7 in PINS:
                        w = (pin(w[0], (yield)), w[1])
                    for rho in range(10, 13):
                        w = _cmul_conj(w, z256)
                        st_h(rho, w)

    def tap_pair(i):
        d = 2 * i

        def ld2(buf, k, pitch, n):
            return jnp.concatenate([buf[k, pl.ds(pitch * d, n), :],
                                    buf[k, pl.ds(pitch * (d + 1), n), :]], axis=0)

        def bc2(k):
            return jnp.concatenate(
                [jnp.broadcast_to(sbuf[k, pl.ds(d + t, 1), :], (8, 128)) for t in range(2)], axis=0)

        zs = [[None] * 4 for _ in range(8)]
        for k in range(2):
            z = (ld2(ebuf, k, ES, 8), ld2(ebuf, 2 + k, ES, 8))
            step = (bc2(k), bc2(2 + k))
            for g in range(8):
                zs[g][k], zs[g][2 + k] = z
                if g < 7:
                    z = _cmul(z, step)
        lo = jnp.concatenate([jnp.concatenate(zs[g], axis=1) for g in range(8)], axis=0).astype(bf16)
        hi = jnp.concatenate([ld2(hbuf, k, HS, 16) for k in range(4)], axis=1).astype(bf16)
        res = lax.dot_general(hi, lo, (((1,), (1,)), ((), ())), preferred_element_type=f32)
        rbuf[pl.ds(RS * d, 16), :] = res[0:16]
        rbuf[pl.ds(RS * (d + 1), 16), :] = res[16:32]

    qscale = float(DH ** -0.5 * np.log2(np.e))
    pad0 = jnp.zeros((32 - DH, BQ), f32)
    one_row = (lax.broadcasted_iota(jnp.int32, (128, BQ), 0) & 31) == DH
    n_marks = 8 * 28 + 4 * 32

    def proj(tb, groups, n_skip):
        first = isinstance(tb, int) and tb == 0
        ts = pl.ds(tb * BQ if isinstance(tb, int) else pl.multiple_of(tb * BQ, BQ), BQ)
        pltpu.make_async_copy(xt_hbm.at[:, ts], xs.at[0:D, ts], sems.at[SEM_X + tb]).wait()
        xi[:, ts] = _pack(xs[:, ts])
        job = powers(groups)
        n_stage = len(PINS) * 4 * len(groups)
        n_mark = n_marks - n_skip
        cnt = {"mark": 0, "stage": 0}

        def pace(val):
            for g in range(val.shape[0] // 16):
                cnt["mark"] += 1
                m = cnt["mark"] - n_skip
                if m == 1:
                    if first:
                        for c in c_p:
                            c.wait()
                    next(job)
                while m > 0 and cnt["stage"] < (m * n_stage + n_mark - 1) // n_mark:
                    cnt["stage"] += 1
                    try:
                        job.send(val[16 * g:16 * g + 8, 0:128])
                    except StopIteration:
                        pass

        def qv(g):
            r = None
            for kt in range(4):
                ks = slice(128 * kt, 128 * (kt + 1))
                kh = slice(64 * kt, 64 * (kt + 1))
                part = jnp.dot(_unpack(wqv[56 * g:56 * (g + 1), ks]), _unpack(xi[kh, ts]),
                               preferred_element_type=f32)
                r = part if r is None else r + part
                pace(part)
            if g < 4:
                qt[g, :, ts] = _pack(_spread(r, pad0) * qscale)
            else:
                v = _pack(jnp.where(one_row, 1.0, _spread(r, pad0)))
                for hh in range(4):
                    vt[4 * (g - 4) + hh, :, ts] = v[16 * hh:16 * (hh + 1)]

        def keys(tt):
            t0 = tb * BQ + 128 * tt
            tsl = pl.ds(t0 if isinstance(t0, int) else pl.multiple_of(t0, 128), 128)
            k = None
            for kt in range(4):
                kh = slice(64 * kt, 64 * (kt + 1))
                part = lax.dot_general(_unpack(xi[kh, tsl]), _unpack(wk[kh, :]),
                                       (((0,), (0,)), ((), ())), preferred_element_type=f32)
                k = part if k is None else k + part
                pace(part)
            kb = _pack(k)
            th = tb * (BQ // 2) + 64 * tt
            tsh = pl.ds(th if isinstance(th, int) else pl.multiple_of(th, 64), 64)
            for c in range(4):
                kp[c, tsh, :] = kb[:, 128 * c:128 * (c + 1)]

        if first:
            for g in range(8):
                qv(g)
                if g == 0:
                    prep_v()
                if g == 1:
                    prep_dt()
                if g == 3:
                    prep_k()
            for tt in range(4):
                keys(tt)
        else:
            for g in range(8):
                qv(g)
                if g % 2 == 1:
                    keys(g // 2)
        assert cnt["stage"] == n_stage

    g0 = G_FIRST
    g1 = (D // 16 - g0) // (S // BQ - 1)
    assert g0 + g1 * (S // BQ - 1) == D // 16
    proj(0, list(range(g0)), NSKIP)

    def proj_body(tb, carry):
        proj(tb, [g0 + (tb - 1) * g1 + g for g in range(g1)], 0)
        return carry

    lax.fori_loop(1, S // BQ, proj_body, 0)

    nq = S // BQ
    nc = S // CK

    def masked_q(c, q0, j):
        parts = []
        if j > 0:
            parts.append(jnp.zeros((32 * j, BQ), bf16))
        parts.append(_unpack(qt[c, 16 * j:16 * (j + 1), pl.ds(q0, BQ)]))
        if j < 3:
            parts.append(jnp.zeros((32 * (3 - j), BQ), bf16))
        return jnp.concatenate(parts, axis=0)

    def unit(i):
        return i // nq, pl.multiple_of((i % nq) * BQ, BQ)

    qm = masked_q(0, 0, 0)
    mp = None
    for kc in range(nc):
        sl = slice(kc * CK, (kc + 1) * CK)
        s = jnp.dot(_unpack(kp[0, kc * CK // 2:(kc + 1) * CK // 2, :]), qm,
                    preferred_element_type=f32)
        s_ref[0, sl, :] = s
        cm = jnp.max(s.reshape(CK // 8, 8, BQ), axis=0)
        mp = cm if mp is None else jnp.maximum(mp, cm)
    m0 = jnp.max(mp, axis=0, keepdims=True)

    n_it = 4 * nq
    s_ref[1, S - CK:S, :] = jnp.zeros((CK, BQ), f32)

    def pv(slot, h, kc, m, acc):
        sl = slice(kc * CK, (kc + 1) * CK)
        p = jnp.exp2(s_ref[slot, sl, :] - m).astype(bf16)
        o = jnp.dot(_unpack(vt[h, :, sl]), p, preferred_element_type=f32)
        return o if acc is None else acc + o

    def normalise(h, q0, acc):
        inv = 1.0 / acc[DH:DH + 1]
        ot[pl.ds(pl.multiple_of(h * 16, 16), 16), pl.ds(q0, BQ)] = _pack(acc * inv)

    def att(side_job, i, carry, last=False, filler=None):
        m_cur, m_prev, acc = carry
        state = {}
        for j in range(4):
            c, q0 = unit(i)
            h = c * 4 + j
            if j > 0:
                hp, q0p = h - 1, q0
            else:
                cp, q0p = unit(jnp.maximum(i - 1, 0))
                hp = cp * 4 + 3
            do_qk = not (last and j == 3)
            if j < 3:
                cn, q0n, jn = c, q0, j + 1
            else:
                cn, q0n = unit(jnp.minimum(i + 1, n_it - 1))
                jn = 0
            slot, nslot = j % 2, (j + 1) % 2
            if do_qk:
                qm = masked_q(cn, q0n, jn)
            mp = None
            for kc in range(nc):
                if do_qk:
                    sl = slice(kc * CK, (kc + 1) * CK)
                    s = jnp.dot(_unpack(kp[cn, kc * CK // 2:(kc + 1) * CK // 2, :]), qm,
                                preferred_element_type=f32)
                    s_ref[nslot, sl, :] = s
                    cm = jnp.max(s.reshape(CK // 8, 8, BQ), axis=0)
                    mp = cm if mp is None else jnp.maximum(mp, cm)
                    side_job(i, j * nc + kc, s, state)
                elif filler is not None:
                    filler(kc)
                if kc == 0:
                    normalise(hp, q0p, pv(nslot, hp, nc - 1, m_prev, acc))
                    acc = None
                else:
                    acc = pv(slot, h, kc - 1, m_cur, acc)
            m_prev = m_cur
            if do_qk:
                m_cur = jnp.max(mp, axis=0, keepdims=True)
        if last:
            normalise(h, q0, pv(1, h, nc - 1, m_prev, acc))
        return m_cur, m_prev, acc

    n_a = n_it // 2
    ppi = (D // 2) // n_a
    pair_at = {(k * 64) // ppi: k for k in range(ppi)}

    def tap_job(i, ci, s, state):
        if ci in pair_at:
            tap_pair(i * ppi + pair_at[ci])

    carry = (m0, jnp.zeros((1, BQ), f32), jnp.zeros((32, BQ), f32))
    carry = lax.fori_loop(0, n_a, lambda i, m: att(tap_job, i, m), carry)

    for c in (c_ds, c_wo, c_u, c_fu, c_gi, c_fk):
        c.wait()
    dsk = jnp.concatenate([jnp.zeros((1, DP - D), f32),
                           dskip_v[...].astype(f32).reshape(1, D)], axis=1)
    odd = (lax.broadcasted_iota(jnp.int32, (8, DP), 1) & 1) == 1
    first = lax.broadcasted_iota(jnp.int32, (8, DP), 0) == 0

    def table(rho, tile):
        raw = rbuf[pl.ds(rho, D, stride=RS), :]
        raw = jnp.concatenate([raw[0:8] + tile * 0.0, raw[8:]], axis=0)
        m = jnp.concatenate([jnp.zeros((DP - D, 128), f32), raw], axis=0)
        mt = m.T
        rows = [jnp.where(odd, mt[16 * g + 8:16 * g + 16], mt[16 * g:16 * g + 8]) for g in range(8)]
        if rho == 0:
            rows[0] = rows[0] + jnp.where(first, dsk, 0.0)
        packed = _pack(jnp.concatenate(rows, axis=0))
        for unit in range(4):
            r0 = 8 * _slot(rho, unit)
            tm[r0:r0 + 8, :] = packed[8 * unit:8 * (unit + 1)]

    def put_spectrum(slab, r):
        for g in range(16):
            for t in range(4):
                r0 = 32 * t + 16 * (g // 8) + (8 if slab >= NB else 0)
                kx[g % 8, slab, r0:r0 + 16, :] = r[16 * g:16 * (g + 1), 128 * t:128 * (t + 1)]

    tm[NLO // 2 * len(HI):NLO // 2 * 14, :] = jnp.zeros((NLO // 2, DP), jnp.int32)
    for j in range(NB):
        r = lax.dot_general(_unpack(fu_ref[...]), us[:, 128 * j:128 * (j + 1)], (((1,), (1,)), ((), ())),
                            preferred_element_type=f32)
        put_spectrum(NB + j, r)
        if j < len(HI):
            table(j, r[0:8, 0:128])
        if j == len(HI):
            wo_r = wo_raw[...].astype(f32)
            wo_r = jnp.concatenate([wo_r[0:8] + r[0:8, 0:1] * 0.0, wo_r[8:]], axis=0)
            wo_r = _respace(wo_r, 0)
            wo2[...] = _pack(jnp.concatenate([wo_r, jnp.zeros((512, DP - D), f32)], axis=1))
    for j in range(NB):
        r = None
        for idx, kt in _FK_INDEX[j]:
            part = jnp.dot(_unpack(fk_ref[idx]), _unpack(tm[64 * kt:64 * (kt + 1), :]),
                           preferred_element_type=f32)
            r = part if r is None else r + part
        put_spectrum(j, r)

    units = [(t, io, hf, p) for t in range(4) for io in range(NB) for hf in range(2)
             for p in range(io + 1)]

    def mac_job(i, ci, s, state, n_chunks=64):
        fg = i - n_a
        if MAC_SKIP:
            if ci % nc < MAC_SKIP:
                return
            ci, n_chunks = ci - MAC_SKIP * (ci // nc + 1), n_chunks - MAC_SKIP * (n_chunks // nc)
        mine = units[(ci * len(units)) // n_chunks:((ci + 1) * len(units)) // n_chunks]
        for m, (t, io, hf, p) in enumerate(mine):
            g = (m * MAC_PINS) // len(mine)
            r0 = 32 * t + 8 * hf
            kr, ki = kx[fg, p, r0:r0 + 8, :], kx[fg, p, r0 + 16:r0 + 24, :]
            ur = kx[fg, NB + io - p, r0 + 8:r0 + 16, :]
            ui = kx[fg, NB + io - p, r0 + 24:r0 + 32, :]
            if m == 0 or ((m - 1) * MAC_PINS) // len(mine) != g:
                g8 = 8 * (g * 16 // MAC_PINS)
                kr = kr + s[g8:g8 + 8, 0:128] * 0.0
            a = kr * ur - ki * ui
            b = kr * ui + ki * ur
            if p == 0:
                state["re"], state["im"] = a, b
            else:
                state["re"], state["im"] = state["re"] + a, state["im"] + b
            if p == io:
                if hf == 0:
                    state["re0"], state["im0"] = state["re"], state["im"]
                else:
                    ls = slice(128 * t, 128 * (t + 1))
                    y0 = fg * 16
                    y0 = y0 if isinstance(y0, int) else pl.multiple_of(y0, 16)
                    yb[io, pl.ds(y0, 8), ls] = _pack(jnp.concatenate(
                        [state["re0"], state["re"]], axis=0))
                    yb[io, pl.ds(y0 + 8, 8), ls] = _pack(jnp.concatenate(
                        [state["im0"], state["im"]], axis=0))

    carry = lax.fori_loop(n_a, n_it - 1, lambda i, m: att(mac_job, i, m), carry)
    lane = lax.broadcasted_iota(jnp.int32, (128, 128), 1)

    def finish(i):
        rows = slice(128 * i, 128 * (i + 1))
        y = jnp.dot(_unpack(gi_ref[...]), _unpack(yb[i]), preferred_element_type=f32)
        a = lax.dot_general(_unpack(ot[:, rows]), _unpack(wo2[...]), (((0,), (0,)), ((), ())),
                            preferred_element_type=f32)
        ob[rows, 0:384] = a[:, 0:384].astype(bf16)
        ob[rows, 384:512] = jnp.where(lane < 64, a[:, 384:512], y[:, 0:128]).astype(bf16)
        ob[rows, 512:896] = y[:, 128:512].astype(bf16)
        copy(ob.at[rows, :], out_hbm.at[rows, :], SEM_O + i).start()

    def filler(kc):
        if kc in FILL_AT:
            finish(FILL_AT.index(kc))

    att(lambda i, ci, s, st: mac_job(i, ci, s, st, 48), n_it - 1, carry, last=True, filler=filler)
    for i in range(len(FILL_AT), NB):
        finish(i)
    for i in range(NB):
        rows = slice(128 * i, 128 * (i + 1))
        copy(ob.at[rows, :], out_hbm.at[rows, :], SEM_O + i).wait()


@jax.jit
def pallas_concat_heads__mha_block__ssm_conv_s4__prompt_kernel(
    A_x: jax.Array,
    A_wqkv: jax.Array,
    A_wo: jax.Array,
    B_u: jax.Array,
    B_A_re: jax.Array,
    B_A_im: jax.Array,
    B_B_re: jax.Array,
    B_B_im: jax.Array,
    B_C_re: jax.Array,
    B_C_im: jax.Array,
    B_log_dt: jax.Array,
    B_Dskip: jax.Array,
):
    vm = pltpu.VMEM
    i32 = jnp.int32
    scratch = [
        vm((D, 3 * D), bf16), vm((D, D), bf16), vm((DP, S), bf16), vm((DP // 2, S), i32),
        vm((6, D, N), bf16),
        vm((D,), bf16), vm((D,), bf16), vm((128, 128), i32), vm((64, 256), i32),
        vm((_NFK, 128, 128), i32),
        vm((D, DP), i32), vm((DP // 2, 512), i32), vm((256, DP), i32),
        vm((4, S // 2, 128), i32), vm((4, 64, S), i32), vm((H, 16, S), i32),
        vm((2, S, BQ), f32), vm((256, S), i32),
        vm((DP, 128), f32), vm((4, ES * D + 16, 128), f32), vm((4, HS * D + 16, 128), f32),
        vm((4, D, 128), f32), vm((RS * D + 16, 128), f32), vm((7 * NLO, DP), i32),
        vm((DP, S), bf16), vm((8, 2 * NB, 160, 128), f32),
        vm((NB, 128, DP), i32), vm((S, 2 * D), bf16),
        pltpu.SemaphoreType.DMA((N_SEM,)),
    ]
    hbm = pl.BlockSpec(memory_space=pl.ANY)
    out = pl.pallas_call(
        _kernel,
        out_shape=jax.ShapeDtypeStruct((S, 2 * D), bf16),
        in_specs=[hbm] * 15,
        out_specs=hbm,
        scratch_shapes=scratch,
        compiler_params=pltpu.CompilerParams(vmem_limit_bytes=110 * 1024 * 1024, flags=FLAGS),
    )(jnp.transpose(A_x, (0, 2, 1)).reshape(D, S), A_wqkv, A_wo,
      jnp.transpose(B_u, (0, 2, 1)).reshape(D, S),
      B_A_re, B_A_im, B_B_re, B_B_im, B_C_re, B_C_im, B_log_dt, B_Dskip,
      jnp.asarray(_pack_host(_FU)), jnp.asarray(_pack_host(_GI)), jnp.asarray(_pack_host(_FK)))
    return out.reshape(1, S, 2 * D)
```
